```python
import jax
import jax.numpy as jnp

def _softmax(x, axis=-1):
    return jax.nn.softmax(x, axis=axis)

def _gelu(x):
    return jax.nn.gelu(x, approximate=True)

def _silu(x):
    return jax.nn.silu(x)

def _sigmoid(x):
    return jax.nn.sigmoid(x)

def _layernorm(x, axis=-1, eps=1e-05):
    m = jnp.mean(x, axis=axis, keepdims=True)
    v = jnp.var(x, axis=axis, keepdims=True)
    return (x - m) / jnp.sqrt(v + eps)

def _scatter_add(tgt, idx, src, axis=0):
    return tgt.at[idx].add(src)

def _segment_sum(src, seg, n):
    return jax.ops.segment_sum(src, seg, n)

class _Rng:

    def __init__(self, key):
        self._k = key

    def _next(self):
        self._k, sub = jax.random.split(self._k)
        return sub

    def normal(self, shape):
        return jax.random.normal(self._next(), shape, dtype=jnp.bfloat16)

    def randint(self, lo, hi, shape):
        return jax.random.randint(self._next(), shape, lo, hi, dtype=jnp.int32)

    def uniform(self, shape, lo=0.0, hi=1.0):
        return jax.random.uniform(self._next(), shape, jnp.bfloat16, lo, hi)

    def permutation(self, n):
        return jax.random.permutation(self._next(), n)
kernel_name = 'gated_mix__ssm_conv_h3__memory_aug_recurrent_mem_tr__prompt'

def setup_inputs():
    _rng = _Rng(jax.random.key(int.from_bytes(__import__("os").urandom(4), "little")))
    _w = lambda a: (lambda t: t.astype(jnp.bfloat16) if jnp.issubdtype(t.dtype, jnp.floating) else t)(jnp.asarray(a))

    def _A_setup():
        B, S, D = (1, 2048, 1024)
        ks = 4
        return {'q': _w((lambda *s: _rng.normal(s) * 0.05)(B, S, D)), 'k': _w((lambda *s: _rng.normal(s) * 0.05)(B, S, D)), 'v': _w((lambda *s: _rng.normal(s) * 0.05)(B, S, D)), 'shift_k': _w((lambda *s: _rng.normal(s) * 0.05)(D, ks) * 0.5), 'ssm_k': _w((lambda *s: _rng.normal(s) * 0.05)(D, S) * (1.0 / S ** 0.5)), 'ssm_D': _w((lambda *s: _rng.normal(s) * 0.05)(D))}
    _A_in = _A_setup()

    def _B_setup():
        B, S, Dm = (1, 2048, 1024)
        H, Dh = (32, 128)
        M, seg = (8, 32)
        seg = min(seg, S)
        S = S // seg * seg
        return {'x': _w((lambda *s: _rng.normal(s) * 0.05)(B, S, Dm)), 'mem0': _w((lambda *s: _rng.normal(s) * 0.05)(B, M, Dm)), 'Wq': _w((lambda *s: _rng.normal(s) * 0.05)(Dm, H, Dh) * Dm ** (-0.5)), 'Wk': _w((lambda *s: _rng.normal(s) * 0.05)(Dm, H, Dh) * Dm ** (-0.5)), 'Wv': _w((lambda *s: _rng.normal(s) * 0.05)(Dm, H, Dh) * Dm ** (-0.5)), 'Wo': _w((lambda *s: _rng.normal(s) * 0.05)(H, Dh, Dm) * (H * Dh) ** (-0.5)), 'seg_len': seg}
    _B_in = _B_setup()
    return {'A_q': _A_in['q'], 'A_k': _A_in['k'], 'A_v': _A_in['v'], 'A_shift_k': _A_in['shift_k'], 'A_ssm_k': _A_in['ssm_k'], 'A_ssm_D': _A_in['ssm_D'], 'B_x': _B_in['x'], 'B_mem0': _B_in['mem0'], 'B_Wq': _B_in['Wq'], 'B_Wk': _B_in['Wk'], 'B_Wv': _B_in['Wv'], 'B_Wo': _B_in['Wo'], 'B_seg_len': _B_in['seg_len'], 'gate_w': _w((lambda *s: _rng.normal(s) * 0.05)(1024))}

def reference(A_q, A_k, A_v, A_shift_k, A_ssm_k, A_ssm_D, B_x, B_mem0, B_Wq, B_Wk, B_Wv, B_Wo, B_seg_len, gate_w):

    def _A_ref(q, k, v, shift_k, ssm_k, ssm_D):
        B, S, D = q.shape
        ks = shift_k.shape[-1]
        k_pad = jnp.pad(k, ((0, 0), (ks - 1, 0), (0, 0)))
        k_shift = jnp.zeros_like(k)
        for t in range(ks):
            k_shift = k_shift + k_pad[:, t:t + S, :] * shift_k[:, ks - 1 - t][None, None, :]
        kv = k_shift * v
        L = 2 * S
        kv_pad = jnp.pad(kv, ((0, 0), (0, S), (0, 0)))
        kf_pad = jnp.pad(ssm_k, ((0, 0), (0, S)))
        kv_f = (lambda x, axes=(-2, -1): jnp.fft.rfft2(x.astype(jnp.float32), axes=axes))(kv_pad[:, None, :, :], axes=(1, 2))
        kf_f = (lambda x, axes=(-2, -1): jnp.fft.rfft2(x.astype(jnp.float32), axes=axes))(kf_pad[:, None, :], axes=(1, 2))
        kf_f = (lambda x, *d: x.transpose(*d))(kf_f, 1, 2, 0)
        y_f = kv_f * kf_f[None, :, :, :]
        y = (lambda x, s, axes=(-2, -1): jnp.fft.irfft2(x, s=s, axes=axes).astype(jnp.bfloat16))(y_f, (1, L), axes=(1, 2))[:, 0, :S, :]
        y = y + kv * ssm_D[None, None, :]
        return q * y

    def _B_ref(x, mem0, Wq, Wk, Wv, Wo, seg_len):
        B, S, Dm = x.shape
        H, Dh = (Wq.shape[1], Wq.shape[2])
        M = mem0.shape[1]
        scale = Dh ** (-0.5)
        n_seg = S // seg_len
        L = M + seg_len
        idx = jnp.arange(L)
        mask = (idx[:, None] < M) | (idx[:, None] >= idx[None, :])
        mem = mem0
        outs = []
        for s in range(n_seg):
            xs = x[:, s * seg_len:(s + 1) * seg_len, :].copy()
            h = jnp.concatenate([mem, xs], axis=1)
            q = jnp.einsum('btd,dhe->bhte', h, Wq)
            k = jnp.einsum('btd,dhe->bhte', h, Wk)
            v = jnp.einsum('btd,dhe->bhte', h, Wv)
            scores = jnp.einsum('bhqe,bhke->bhqk', q, k) * scale
            scores = jnp.where(mask[None, None], scores, -1000000000.0)
            p = _softmax(scores, axis=-1)
            o = jnp.einsum('bhqk,bhke->bhqe', p, v)
            o = jnp.einsum('bhte,hed->btd', o, Wo)
            mem = o[:, :M, :].copy()
            outs.append(o[:, M:, :])
        return jnp.concatenate(outs, axis=1)
    x = A_q
    g = _sigmoid((x * gate_w).sum(-1, keepdims=True))
    a = _A_ref(x, A_k, A_v, A_shift_k, A_ssm_k, A_ssm_D)
    b = _B_ref(x, B_mem0, B_Wq, B_Wk, B_Wv, B_Wo, B_seg_len)
    return g * a + (1 - g) * b
```

```python
import functools
import numpy as np
import jax
import jax.numpy as jnp
import jax.experimental.pallas as pl
import jax.experimental.pallas.tpu as pltpu

S = 2048
D = 1024
H = 32
E = 128
M = 8
SEG = 32
NSEG = S // SEG
C = 128
NB = S // C
NT = D // 128
KS = 4
L = M + SEG
LP = 48

BF = jnp.bfloat16
F32 = jnp.float32


def _dft_consts():
    f = np.arange(C, dtype=np.float64)[:, None] + 0.5
    c = np.arange(C, dtype=np.float64)[None, :]
    th = 2.0 * np.pi * f * c / (2 * C)
    fwd = np.concatenate([np.cos(th), -np.sin(th)], axis=0)
    inv = np.concatenate([np.cos(th).T, -np.sin(th).T], axis=1) / C * 128.0
    return fwd.astype(np.float32), inv.astype(np.float32)


_FWD, _INV = _dft_consts()
_NT_DIMS = (((1,), (1,)), ((), ()))


def _dot(a, b):
    return jnp.dot(a, b, preferred_element_type=F32)


def _dot_nt(a, b):
    return jax.lax.dot_general(a, b, _NT_DIMS, preferred_element_type=F32)


def _kernel(
    shift_ref, ssmd_ref, gw_ref, mem0_ref, fwd_ref, inv_ref,
    x_hbm, k_hbm, v_hbm, sk_hbm, wq_hbm, wk_hbm, wv_hbm, wo_hbm,
    out_hbm,
    xb, kb, vb, skb,
    gab,
    omg,
    xs, ks, zs, kvs,
    wst,
    wqkv,
    wob,
    ring,
    l1,
    ebuf, obuf,
    outb,
    sem_a, sem_w, sem_o,
):
    def a_copies(t):
        return [
            pltpu.make_async_copy(x_hbm.at[:, pl.ds(t * 128, 128)], xb.at[t], sem_a.at[0, t]),
            pltpu.make_async_copy(k_hbm.at[:, pl.ds(t * 128, 128)], kb.at[t], sem_a.at[1, t]),
            pltpu.make_async_copy(v_hbm.at[:, pl.ds(t * 128, 128)], vb.at[t], sem_a.at[2, t]),
            pltpu.make_async_copy(sk_hbm.at[pl.ds(t * 128, 128), :], skb.at[t], sem_a.at[3, t]),
        ]

    for t in range(NT):
        a_copies(t)[0].start()
    for t in range(NT):
        for c in a_copies(t)[1:]:
            c.start()

    whbm = (wq_hbm, wk_hbm, wv_hbm)

    def w_copy(i):
        return pltpu.make_async_copy(whbm[i], wst.at[i], sem_w.at[i])

    def wo_copy(j):
        return pltpu.make_async_copy(wo_hbm.at[:, pl.ds(j * 128, 128)], wob.at[j], sem_w.at[3 + j])

    for t in range(NT):
        a_copies(t)[0].wait()
    gw = gw_ref[...].astype(F32)

    def gate_body(i, carry):
        r0 = pl.multiple_of(i * 128, 128)
        acc = None
        for t in range(NT):
            p = xb[t, pl.ds(r0, 128), :].astype(F32) * gw[:, t * 128:(t + 1) * 128]
            acc = p if acc is None else acc + p
        lg = jnp.sum(acc, axis=-1, keepdims=True)
        g = jax.nn.sigmoid(lg)
        omg[pl.ds(r0, 128), :] = jnp.broadcast_to(1.0 - g, (128, 128))
        return carry

    jax.lax.fori_loop(0, S // 128, gate_body, 0)

    fwd = fwd_ref[...]
    inv = inv_ref[...]
    shift = shift_ref[...].astype(F32)
    ssmd = ssmd_ref[...].astype(F32)
    rowpar = jax.lax.broadcasted_iota(jnp.int32, (8, 128), 0)
    sgn = jnp.where((rowpar & 1) == 0, 1.0, -1.0).astype(F32)

    for t in range(NT):
        if t == 2:
            for i in range(3):
                w_copy(i).start()
            for j in range(NT):
                wo_copy(j).start()
        cps = a_copies(t)
        cps[1].wait()
        cps[2].wait()
        cps[3].wait()
        sh = [shift[q:q + 1, t * 128:(t + 1) * 128] for q in range(KS)]
        dd = ssmd[:, t * 128:(t + 1) * 128]

        def fwd_body(j, carry):
            r0 = pl.multiple_of(j * C, C)
            kcur = kb[t, pl.ds(r0, C), :].astype(F32)
            rp = pl.multiple_of(jnp.maximum(r0 - 16, 0), 16)
            kprev = kb[t, pl.ds(rp, 16), :].astype(F32)
            kprev = jnp.where(j > 0, kprev, 0.0)[8:16]
            kext = jnp.concatenate([kprev, kcur], axis=0)
            ksh = kcur * sh[0]
            for q in range(1, KS):
                ksh = ksh + kext[8 - q:8 - q + C] * sh[q]
            kv = (ksh * vb[t, pl.ds(r0, C), :].astype(F32)).astype(BF)
            kvs[pl.ds(r0, C), :] = kv.astype(F32)
            xs[j] = _dot(fwd, kv)
            ks[j] = _dot_nt(fwd, skb[t, :, pl.ds(r0, C)])
            return carry

        jax.lax.fori_loop(0, NB, fwd_body, 0)

        def conv_body(g, carry):
            f0 = pl.multiple_of(g * 8, 8)
            xr = [xs[j, pl.ds(f0, 8), :] for j in range(NB)]
            xi = [xs[j, pl.ds(C + f0, 8), :] for j in range(NB)]
            kr = [ks[j, pl.ds(f0, 8), :] for j in range(NB)]
            ki = [ks[j, pl.ds(C + f0, 8), :] for j in range(NB)]
            pr = pi = None
            for i in range(NB):
                yr = xr[i] * kr[0] - xi[i] * ki[0]
                yi = xr[i] * ki[0] + xi[i] * kr[0]
                for j in range(1, i + 1):
                    yr = yr + (xr[i - j] * kr[j] - xi[i - j] * ki[j])
                    yi = yi + (xr[i - j] * ki[j] + xi[i - j] * kr[j])
                if i == 0:
                    zr, zi = yr, yi
                else:
                    zr = yr - sgn * pi
                    zi = yi + sgn * pr
                pr, pi = yr, yi
                zs[i, pl.ds(f0, 8), :] = zr
                zs[i, pl.ds(C + f0, 8), :] = zi
            return carry

        jax.lax.fori_loop(0, C // 8, conv_body, 0)

        def inv_body(i, carry):
            r0 = pl.multiple_of(i * C, C)
            y = _dot(inv, zs[i].astype(BF)) * (1.0 / 128.0)
            y = y.astype(BF).astype(F32) + kvs[pl.ds(r0, C), :] * dd
            a = xb[t, pl.ds(r0, C), :].astype(F32) * y
            g = 1.0 - omg[pl.ds(r0, C), :]
            gab[t, pl.ds(r0, C), :] = g * a
            return carry

        jax.lax.fori_loop(0, NB, inv_body, 0)

    for i in range(3):
        w_copy(i).wait()

        def rel_body(b, carry):
            d0 = pl.multiple_of(b * 16, 16)
            wqkv[i * H:(i + 1) * H, pl.ds(d0, 16), :] = jnp.swapaxes(wst[i, pl.ds(d0, 16), :, :], 0, 1)
            return carry

        jax.lax.fori_loop(0, D // 16, rel_body, 0)
    for j in range(NT):
        wo_copy(j).wait()

    ring[...] = jnp.zeros(ring.shape, BF)
    ebuf[...] = jnp.zeros(ebuf.shape, BF)
    l1[...] = jnp.zeros(l1.shape, BF)

    xl = jnp.concatenate([xb[t, 0:64, :] for t in range(NT)], axis=1)
    for c in range(96):
        y = _dot(xl, wqkv[c]).astype(BF)
        ring[0, c, 8:40, :] = y[0:32]
        ring[1, c, 8:40, :] = y[32:64]

    r = jax.lax.broadcasted_iota(jnp.int32, (L, 128), 0)
    cidx = jax.lax.broadcasted_iota(jnp.int32, (L, 128), 1)
    amask = ((r < M) | (r >= cidx)) & (cidx < L)
    scale = float(E) ** -0.5

    def attention(slot, h):
        q = ring[slot, h, :, :]
        k = ring[slot, H + h, :, :]
        v = ring[slot, 2 * H + h, :, :]
        s = _dot_nt(q, k)[0:L] * scale
        s = jnp.where(amask[:, 0:LP], s, -1e9)
        m = jnp.max(s, axis=-1, keepdims=True)
        p = jnp.exp(s - m)
        den = jnp.sum(p, axis=-1, keepdims=True)
        p = p / den
        pz = jnp.concatenate([p, jnp.zeros((LP - L, LP), F32)], axis=0).astype(BF)
        return _dot(pz, v)[0:L]

    def combine(j, row0, b):
        n = b.shape[0]
        o = gab[j, pl.ds(row0, n), :] + omg[pl.ds(row0, n), :] * b.astype(BF).astype(F32)
        outb[j, pl.ds(row0, n), :] = o.astype(BF)

    def put_mem(mem):
        for t in range(NT):
            l1[t, 0:8, :] = mem[:, t * 128:(t + 1) * 128].astype(BF)

    put_mem(mem0_ref[...].astype(F32))

    def pair_body(p, carry):
        s0 = 2 * p
        sl0 = jax.lax.rem(s0, 4)
        sl1 = sl0 + 1
        sl2 = jax.lax.rem(s0 + 2, 4)
        sl3 = sl2 + 1
        ra = pl.multiple_of(jnp.minimum(s0 + 2, NSEG - 2) * SEG, SEG)
        rb = pl.multiple_of(ra + SEG, SEG)

        for t in range(NT):
            l1[t, 8:40, :] = xb[t, pl.ds(ra, SEG), :]
            l1[t, 40:48, :] = xb[t, pl.ds(rb + 24, 8), :]
        lhs = jnp.concatenate([l1[t] for t in range(NT)], axis=1)
        for h in range(H):
            for w in range(3):
                c = w * H + h
                y = _dot(lhs, wqkv[c]).astype(BF)
                ring[sl0, c, 0:8, :] = y[0:8]
                ring[sl2, c, 8:40, :] = y[8:40]
                ring[sl3, c, 32:40, :] = y[40:48]
        for h in range(H):
            o = attention(sl0, h).astype(BF)
            ebuf[h, 0:40, :] = o
        lhs = jnp.concatenate([ebuf[h] for h in range(H)], axis=1)
        ys = []
        for j in range(NT):
            y = _dot(lhs, wob[j])
            ys.append(y[0:8])
            combine(j, pl.multiple_of(s0 * SEG, SEG), y[8:40])

            @pl.when(p > 0)
            def _():
                combine(j, pl.multiple_of(s0 * SEG - 8, 8), y[40:48])
        put_mem(jnp.concatenate(ys, axis=1))

        for t in range(NT):
            l1[t, 8:32, :] = xb[t, pl.ds(rb, 24), :]
        lhs = jnp.concatenate([l1[t, 0:32, :] for t in range(NT)], axis=1)
        for h in range(H):
            for w in range(3):
                c = w * H + h
                y = _dot(lhs, wqkv[c]).astype(BF)
                ring[sl1, c, 0:8, :] = y[0:8]
                ring[sl3, c, 8:32, :] = y[8:32]
        for h in range(H):
            o = attention(sl1, h).astype(BF)
            obuf[h, :, :] = o[0:32]
            ebuf[h, 40:48, :] = o[32:40]
        lhs = jnp.concatenate([obuf[h] for h in range(H)], axis=1)
        ys = []
        for j in range(NT):
            y = _dot(lhs, wob[j])
            ys.append(y[0:8])
            combine(j, pl.multiple_of((s0 + 1) * SEG, SEG), y[8:32])
        put_mem(jnp.concatenate(ys, axis=1))
        return carry

    jax.lax.fori_loop(0, NSEG // 2, pair_body, 0)

    lhs = jnp.concatenate([ebuf[h, 32:48, :] for h in range(H)], axis=1)
    for j in range(NT):
        y = _dot(lhs, wob[j])
        combine(j, S - 8, y[8:16])

    ocp = [pltpu.make_async_copy(outb.at[j], out_hbm.at[:, pl.ds(j * 128, 128)], sem_o.at[j]) for j in range(NT)]
    for c in ocp:
        c.start()
    for c in ocp:
        c.wait()


@functools.partial(jax.jit, static_argnames=("B_seg_len",))
def pallas_gated_mix__ssm_conv_h3__memory_aug_recurrent_mem_tr__prompt_kernel(
    A_q, A_k, A_v, A_shift_k, A_ssm_k, A_ssm_D, B_x, B_mem0, B_Wq, B_Wk, B_Wv, B_Wo, B_seg_len, gate_w,
):
    del B_x
    assert A_q.shape == (1, S, D) and B_seg_len == SEG and B_mem0.shape == (1, M, D)
    assert B_Wq.shape == (D, H, E) and A_shift_k.shape == (D, KS)
    vm = pl.BlockSpec(memory_space=pltpu.VMEM)
    hbm = pl.BlockSpec(memory_space=pl.ANY)
    out = pl.pallas_call(
        _kernel,
        out_shape=jax.ShapeDtypeStruct((S, D), BF),
        in_specs=[vm] * 6 + [hbm] * 8,
        out_specs=hbm,
        scratch_shapes=[
            pltpu.VMEM((NT, S, 128), BF), pltpu.VMEM((NT, S, 128), BF), pltpu.VMEM((NT, S, 128), BF),
            pltpu.VMEM((NT, 128, S), BF),
            pltpu.VMEM((NT, S, 128), F32),
            pltpu.VMEM((S, 128), F32),
            pltpu.VMEM((NB, 2 * C, 128), F32), pltpu.VMEM((NB, 2 * C, 128), F32), pltpu.VMEM((NB, 2 * C, 128), F32),
            pltpu.VMEM((S, 128), F32),
            pltpu.VMEM((3, D, H, E), BF),
            pltpu.VMEM((3 * H, D, E), BF),
            pltpu.VMEM((NT, H * E, 128), BF),
            pltpu.VMEM((4, 3 * H, LP, E), BF),
            pltpu.VMEM((NT, LP, 128), BF),
            pltpu.VMEM((H, LP, E), BF), pltpu.VMEM((H, 32, E), BF),
            pltpu.VMEM((NT, S, 128), BF),
            pltpu.SemaphoreType.DMA((4, NT)), pltpu.SemaphoreType.DMA((3 + NT,)), pltpu.SemaphoreType.DMA((NT,)),
        ],
        compiler_params=pltpu.CompilerParams(vmem_limit_bytes=124 * 1024 * 1024),
    )(
        A_shift_k.T, A_ssm_D.reshape(1, D), gate_w.reshape(1, D), B_mem0.reshape(M, D),
        jnp.asarray(_FWD, BF), jnp.asarray(_INV, BF),
        A_q.reshape(S, D), A_k.reshape(S, D), A_v.reshape(S, D), A_ssm_k,
        B_Wq, B_Wk, B_Wv, B_Wo.reshape(H * E, D),
    )
    return out.reshape(1, S, D)
```

```python
import functools
import numpy as np
import jax
import jax.numpy as jnp
import jax.experimental.pallas as pl
import jax.experimental.pallas.tpu as pltpu

S = 2048
D = 1024
H = 32
E = 128
M = 8
SEG = 32
NSEG = S // SEG
C = 128
NB = S // C
NT = D // 128
KS = 4
L = M + SEG
LP = 48

BF = jnp.bfloat16
LAG_E = 4
LAG_O = 5
G = 32
DMA_ORDER = ('0', '1', '2', '3', '4', '5', '6', '7', 'x', 'w0', 'w1', 'w2')
MS = 64
GAUSS = 0
PREP_AT = (7, 8, 9)
UNROLL_G = 0
UF = 2
UI = 2
F32 = jnp.float32


def _dft_consts():
    f = np.arange(C, dtype=np.float64)[:, None] + 0.5
    c = np.arange(C, dtype=np.float64)[None, :]
    th = 2.0 * np.pi * f * c / (2 * C)
    fwd = np.concatenate([np.cos(th), -np.sin(th)], axis=0)
    inv = np.concatenate([np.cos(th).T, -np.sin(th).T], axis=1) / C
    return fwd.astype(np.float32), inv.astype(np.float32)


_FWD, _INV = _dft_consts()
_NT_DIMS = (((1,), (1,)), ((), ()))


def _dot(a, b):
    return jnp.dot(a, b, preferred_element_type=F32)


def _dot_nt(a, b):
    return jax.lax.dot_general(a, b, _NT_DIMS, preferred_element_type=F32)


def _kernel(
    zero_ref, shift_ref, ssmd_ref, gw_ref, mem0_ref, fwd_ref, inv_ref,
    x_hbm, k_hbm, v_hbm, sk_hbm, wq_hbm, wk_hbm, wv_hbm, wo_hbm,
    out_hbm,
    xb, kb, vb, skb,
    yb, kvb,
    kf,
    xsa, ksa, zsa, xsb, ksb, zsb,
    wst,
    wqkv,
    wob,
    ring,
    left,
    ebuf,
    mqkv,
    hyb,
    outb,
    sem_a, sem_w, sem_o,
):
    def a_copies(t):
        return [
            pltpu.make_async_copy(x_hbm.at[:, pl.ds(t * 128, 128)], xb.at[t], sem_a.at[0, t]),
            pltpu.make_async_copy(k_hbm.at[:, pl.ds(t * 128, 128)], kb.at[t], sem_a.at[1, t]),
            pltpu.make_async_copy(v_hbm.at[:, pl.ds(t * 128, 128)], vb.at[t], sem_a.at[2, t]),
            pltpu.make_async_copy(sk_hbm.at[pl.ds(t * 128, 128), :], skb.at[t], sem_a.at[3, t]),
        ]

    whbm = (wq_hbm, wk_hbm, wv_hbm)
    WCH = 4
    DC = D // WCH

    def w_copy(i, c):
        return pltpu.make_async_copy(whbm[i].at[pl.ds(c * DC, DC)], wst.at[i, pl.ds(c * DC, DC)], sem_w.at[i * WCH + c])

    def wo_copy(j):
        return pltpu.make_async_copy(wo_hbm.at[:, pl.ds(j * 128, 128)], wob.at[j], sem_w.at[3 * WCH + j])

    def start_a(t):
        for c in a_copies(t)[1:]:
            c.start()

    def start_w(i):
        for c in range(WCH):
            w_copy(i, c).start()

    def start_x():
        for t in range(NT):
            a_copies(t)[0].start()

    for item in DMA_ORDER:
        if item == 'x':
            start_x()
        elif item[0] == 'w':
            start_w(int(item[1]))
        else:
            start_a(int(item))
    for j in range(NT):
        wo_copy(j).start()

    def relayout_blocks(i, it):
        for b in range(4):
            d0 = pl.multiple_of(it * 64 + b * 16, 16)
            wqkv[i * H:(i + 1) * H, pl.ds(d0, 16), :] = jnp.swapaxes(wst[i, pl.ds(d0, 16), :, :], 0, 1)

    def first_pass(i):
        if i == 0:
            for t in range(NT):
                a_copies(t)[0].wait()
        xl = jnp.concatenate([xb[t, 0:64, :] for t in range(NT)], axis=1)
        for h in range(H):
            c = i * H + h
            y = _dot(xl, wqkv[c]).astype(BF)
            ring[0, c, :, :] = y[0:32]
            ring[1, c, :, :] = y[32:64]

    fwd = fwd_ref[...]
    inv = inv_ref[...]
    shift = shift_ref[...].astype(F32)
    rowpar = jax.lax.broadcasted_iota(jnp.int32, (8, 128), 0)
    sgn = jnp.where((rowpar & 1) == 0, 1.0, -1.0).astype(F32)

    xbufs = ((xsa, ksa, zsa), (xsb, ksb, zsb))

    def fwd_block(t, j):
        xs, ks, _ = xbufs[t % 2]
        sh = [shift[q:q + 1, t * 128:(t + 1) * 128] for q in range(KS)]
        r0 = pl.multiple_of(j * C, C)
        kcur = kb[t, pl.ds(r0, C), :].astype(F32)
        rp = pl.multiple_of(jnp.maximum(r0 - 16, 0), 16)
        kprev = kb[t, pl.ds(rp, 16), :].astype(F32)
        kf[t % 2, 0:8, :] = jnp.where(j > 0, kprev[8:16], 0.0)
        kf[t % 2, 8:8 + C, :] = kcur
        ksh = kcur * sh[0]
        for q in range(1, KS):
            ksh = ksh + kf[t % 2, 8 - q:8 - q + C, :] * sh[q]
        kvf = ksh * vb[t, pl.ds(r0, C), :].astype(F32)
        kv = kvf.astype(BF)
        xs[j] = jnp.concatenate([_dot(fwd[i * MS:(i + 1) * MS], kv) for i in range(2 * C // MS)], axis=0)
        skt = skb[t, :, pl.ds(r0, C)]
        ks[j] = jnp.concatenate([_dot_nt(fwd[i * MS:(i + 1) * MS], skt) for i in range(2 * C // MS)], axis=0)
        kvb[t, pl.ds(r0, C), :] = kv

    def conv_group(t, g):
        xs, ks, zs = xbufs[t % 2]
        f0 = pl.multiple_of(g * 8, 8)
        xr = [xs[j, pl.ds(f0, 8), :] for j in range(NB)]
        xi = [xs[j, pl.ds(C + f0, 8), :] for j in range(NB)]
        kr = [ks[j, pl.ds(f0, 8), :] for j in range(NB)]
        ki = [ks[j, pl.ds(C + f0, 8), :] for j in range(NB)]
        if GAUSS:
            xs_ = [xr[j] + xi[j] for j in range(NB)]
            kd = [ki[j] - kr[j] for j in range(NB)]
            ke = [ki[j] + kr[j] for j in range(NB)]
        pr = pi = None
        for i in range(NB):
            if GAUSS:
                a1 = xs_[i] * kr[0]
                a2 = xr[i] * kd[0]
                a3 = xi[i] * ke[0]
                for j in range(1, i + 1):
                    a1 = a1 + xs_[i - j] * kr[j]
                    a2 = a2 + xr[i - j] * kd[j]
                    a3 = a3 + xi[i - j] * ke[j]
                yr = a1 - a3
                yi = a1 + a2
            else:
                yr = xr[i] * kr[0] - xi[i] * ki[0]
                yi = xr[i] * ki[0] + xi[i] * kr[0]
                for j in range(1, i + 1):
                    yr = yr + (xr[i - j] * kr[j] - xi[i - j] * ki[j])
                    yi = yi + (xr[i - j] * ki[j] + xi[i - j] * kr[j])
            if i == 0:
                zr, zi = yr, yi
            else:
                zr = yr - sgn * pi
                zi = yi + sgn * pr
            pr, pi = yr, yi
            zs[i, pl.ds(f0, 8), :] = zr
            zs[i, pl.ds(C + f0, 8), :] = zi

    def inv_block(t, i):
        zs = xbufs[t % 2][2]
        r0 = pl.multiple_of(i * C, C)
        zb = zs[i].astype(BF)
        y = jnp.concatenate([_dot(inv[m * MS:(m + 1) * MS], zb) for m in range(C // MS)], axis=0)
        yb[t, pl.ds(r0, C), :] = y.astype(BF)

    for st in range(NT + 2):
        if st < NT:
            cps = a_copies(st)
            cps[1].wait()
            cps[2].wait()
            cps[3].wait()
        if st in PREP_AT:
            for c in range(WCH):
                w_copy(PREP_AT.index(st), c).wait()

        def stage_body(i, carry):
            if st in PREP_AT:
                relayout_blocks(PREP_AT.index(st), i)
            if 0 <= st - 2 < NT:
                inv_block(st - 2, i)
            if 0 <= st - 1 < NT:
                conv_group(st - 1, i)
            if st < NT:
                fwd_block(st, i)
            return carry

        jax.lax.fori_loop(0, NB, stage_body, 0)
    for i in range(3):
        first_pass(i)

    for j in range(NT):
        wo_copy(j).wait()

    left[...] = jnp.zeros(left.shape, F32)

    r = jax.lax.broadcasted_iota(jnp.int32, (L, LP), 0)
    cidx = jax.lax.broadcasted_iota(jnp.int32, (L, LP), 1)
    amask = (cidx < L) & ((cidx >= SEG) | (r >= SEG) | (cidx <= r))
    LOG2E = 1.4426950408889634
    scale2 = float(E) ** -0.5 * LOG2E
    neg2 = -1e9 * LOG2E
    z8 = jnp.zeros((8, 128), F32)

    def attention(q, k, v):
        s = _dot_nt(q, k)[0:L]
        s = jnp.where(amask, s * scale2, neg2)
        m = jnp.max(s, axis=-1, keepdims=True)
        p = jnp.exp2(s - m)
        den = jnp.sum(p, axis=-1, keepdims=True)
        pz = jnp.concatenate([p, jnp.zeros((LP - L, LP), F32)], axis=0).astype(BF)
        return _dot(pz, v)[0:L] * (1.0 / den)

    def gate(row0, n):
        acc = None
        for t in range(NT):
            p = xb[t, pl.ds(row0, n), :].astype(F32) * gw_ref[:, t * 128:(t + 1) * 128].astype(F32)
            acc = p if acc is None else acc + p
        return jax.nn.sigmoid(jnp.sum(acc, axis=-1, keepdims=True))

    def combine(j, row0, b, g):
        n = b.shape[0]
        rows = pl.ds(row0, n)
        dd = ssmd_ref[:, j * 128:(j + 1) * 128].astype(F32)
        a = xb[j, rows, :].astype(F32) * (yb[j, rows, :].astype(F32) + kvb[j, rows, :].astype(F32) * dd)
        outb[j, rows, :] = (g * a + (1.0 - g) * b).astype(BF)

    NG = H // G

    def step(even, mem, s, sl, slA, slB, ra, rb):
        nrow = LP if even else 32
        for t in range(NT):
            mt = mem[:, t * 128:(t + 1) * 128]
            extra = xb[t, pl.ds(rb + (24 if even else 16), 8), :].astype(F32)
            hyb[t, :, :] = jnp.concatenate([mt, extra], axis=0).astype(BF)

        def load_lhs():
            parts = []
            for t in range(NT):
                main = xb[t, pl.ds(ra, SEG), :] if even else xb[t, pl.ds(rb, 16), :]
                parts.append(jnp.concatenate([main, hyb[t]], axis=0))
            return jnp.concatenate(parts, axis=1)

        def proj(lhs, h):
            for w in range(3):
                c = w * H + h
                y = _dot(lhs, wqkv[c])
                if even:
                    ring[slA, c, :, :] = y[0:32].astype(BF)
                    ring[slB, c, 24:32, :] = y[40:48].astype(BF)
                    m8 = y[32:40]
                else:
                    ring[slB, c, 0:16, :] = y[0:16].astype(BF)
                    ring[slB, c, 16:24, :] = y[24:32].astype(BF)
                    m8 = y[16:24]
                mqkv[c, :, :] = jnp.concatenate([m8, z8], axis=0).astype(BF)

        def att_load(h):
            return [jnp.concatenate([ring[sl, w * H + h, :, :], mqkv[w * H + h, :, :]], axis=0) for w in range(3)]

        def att(h, qkv):
            o = attention(*qkv)
            if even:
                ebuf[h, :, :] = jnp.concatenate([o, left[h]], axis=0).astype(BF)
            else:
                ebuf[h, 0:32, :] = jnp.concatenate([o[0:16], o[32:40], o[16:24]], axis=0).astype(BF)
                left[h] = o[24:32]

        lhs0 = load_lhs()
        for h in range(G):
            proj(lhs0, h)

        def group_body(g, carry):
            hp = (g - 1) * G
            ins = [att_load(hp + i) for i in range(G)]
            lhs = load_lhs()
            for i in range(G):
                att(hp + i, ins[i])
            for i in range(G):
                proj(lhs, g * G + i)
            return carry

        if NG > 1:
            if UNROLL_G:
                for g in range(1, NG):
                    @pl.when(zero_ref[0] == 0)
                    def _():
                        group_body(g, 0)
            else:
                jax.lax.fori_loop(1, NG, group_body, 0)

        hp = (NG - 1) * G
        ins = [att_load(hp + i) for i in range(G)]
        for i in range(G):
            att(hp + i, ins[i])

        ka = hp * E
        ys = []
        r_cur = pl.multiple_of(s * SEG, SEG)
        if even:
            r_prev = pl.multiple_of(jax.lax.rem(s * SEG + (S - 8), S), 8)
            g_cur = gate(r_cur, 32)
            g_prev = gate(r_prev, 8)
        else:
            r_hi = pl.multiple_of(s * SEG + 16, 8)
            g_cur = gate(r_cur, 16)
            g_hi = gate(r_hi, 8)
        if ka > 0:
            lhsa = jnp.concatenate([ebuf[h, 0:nrow, :] for h in range(hp)], axis=1)
        lhsb = jnp.concatenate([ebuf[h, 0:nrow, :] for h in range(hp, H)], axis=1)
        for j in range(NT):
            y = _dot(lhsb, wob[j, ka:H * E, :])
            if ka > 0:
                y = _dot(lhsa, wob[j, 0:ka, :]) + y
            if even:
                ys.append(y[32:40])
                combine(j, r_cur, y[0:32], g_cur)
                combine(j, r_prev, y[40:48], g_prev)
            else:
                ys.append(y[16:24])
                combine(j, r_cur, y[0:16], g_cur)
                combine(j, r_hi, y[24:32], g_hi)
        return jnp.concatenate(ys, axis=1).astype(BF).astype(F32)

    NOC = 4
    RC = S // NOC

    def out_copy(q, j):
        return pltpu.make_async_copy(outb.at[j, pl.ds(q * RC, RC), :],
                                     out_hbm.at[pl.ds(q * RC, RC), pl.ds(j * 128, 128)], sem_o.at[q, j])

    def pair_body(p, mem):
        for q in range(NOC - 1):
            @pl.when(p == (q + 1) * (NSEG // 2 // NOC) + 1)
            def _():
                for j in range(NT):
                    out_copy(q, j).start()

        s0 = 2 * p
        sl0 = jax.lax.rem(s0, 4)
        sl2 = jax.lax.rem(s0 + 2, 4)
        ra = pl.multiple_of(jnp.minimum(s0 + 2, NSEG - 2) * SEG, SEG)
        rb = pl.multiple_of(ra + SEG, SEG)
        mem = step(True, mem, s0, sl0, sl2, sl2 + 1, ra, rb)
        mem = step(False, mem, s0 + 1, sl0 + 1, sl2, sl2 + 1, ra, rb)
        return mem

    jax.lax.fori_loop(0, NSEG // 2, pair_body, mem0_ref[...].astype(F32))

    g_last = gate(S - 8, 8)
    lhs = jnp.concatenate([jnp.concatenate([left[h], z8], axis=0).astype(BF) for h in range(H)], axis=1)
    for j in range(NT):
        y = _dot(lhs, wob[j])
        combine(j, S - 8, y[0:8], g_last)

    for j in range(NT):
        out_copy(NOC - 1, j).start()
    for q in range(NOC):
        for j in range(NT):
            out_copy(q, j).wait()


@functools.partial(jax.jit, static_argnames=("B_seg_len",))
def pallas_gated_mix__ssm_conv_h3__memory_aug_recurrent_mem_tr__prompt_kernel(
    A_q, A_k, A_v, A_shift_k, A_ssm_k, A_ssm_D, B_x, B_mem0, B_Wq, B_Wk, B_Wv, B_Wo, B_seg_len, gate_w,
):
    del B_x
    assert A_q.shape == (1, S, D) and B_seg_len == SEG and B_mem0.shape == (1, M, D)
    assert B_Wq.shape == (D, H, E) and A_shift_k.shape == (D, KS)
    vm = pl.BlockSpec(memory_space=pltpu.VMEM)
    hbm = pl.BlockSpec(memory_space=pl.ANY)
    out = pl.pallas_call(
        _kernel,
        out_shape=jax.ShapeDtypeStruct((S, D), BF),
        in_specs=[pl.BlockSpec(memory_space=pltpu.SMEM)] + [vm] * 6 + [hbm] * 8,
        out_specs=hbm,
        scratch_shapes=[
            pltpu.VMEM((NT, S, 128), BF), pltpu.VMEM((NT, S, 128), BF), pltpu.VMEM((NT, S, 128), BF),
            pltpu.VMEM((NT, 128, S), BF),
            pltpu.VMEM((NT, S, 128), BF), pltpu.VMEM((NT, S, 128), BF),
            pltpu.VMEM((2, 8 + C, 128), F32),
            pltpu.VMEM((NB, 2 * C, 128), F32), pltpu.VMEM((NB, 2 * C, 128), F32), pltpu.VMEM((NB, 2 * C, 128), F32),
            pltpu.VMEM((NB, 2 * C, 128), F32), pltpu.VMEM((NB, 2 * C, 128), F32), pltpu.VMEM((NB, 2 * C, 128), F32),
            pltpu.VMEM((3, D, H, E), BF),
            pltpu.VMEM((3 * H, D, E), BF),
            pltpu.VMEM((NT, H * E, 128), BF),
            pltpu.VMEM((4, 3 * H, SEG, E), BF),
            pltpu.VMEM((H, 8, E), F32),
            pltpu.VMEM((H, LP, E), BF),
            pltpu.VMEM((3 * H, 16, E), BF),
            pltpu.VMEM((NT, 16, 128), BF),
            pltpu.VMEM((NT, S, 128), BF),
            pltpu.SemaphoreType.DMA((4, NT)), pltpu.SemaphoreType.DMA((12 + NT,)), pltpu.SemaphoreType.DMA((4, NT)),
        ],
        compiler_params=pltpu.CompilerParams(vmem_limit_bytes=124 * 1024 * 1024),
    )(
        np.zeros((1,), np.int32), A_shift_k.T, A_ssm_D.reshape(1, D), gate_w.reshape(1, D), B_mem0.reshape(M, D),
        jnp.asarray(_FWD, BF), jnp.asarray(_INV, BF),
        A_q.reshape(S, D), A_k.reshape(S, D), A_v.reshape(S, D), A_ssm_k,
        B_Wq, B_Wk, B_Wv, B_Wo.reshape(H * E, D),
    )
    return out.reshape(1, S, D)
```

```python
import functools
import numpy as np
import jax
import jax.numpy as jnp
import jax.experimental.pallas as pl
import jax.experimental.pallas.tpu as pltpu

S = 2048
D = 1024
H = 32
E = 128
M = 8
SEG = 32
NSEG = S // SEG
C = 256
NB = S // C
NT = D // 128
KS = 4
L = M + SEG
LP = 48

BF = jnp.bfloat16
G = 32
DMA_ORDER = ('0', '1', '2', '3', '4', '5', '6', '7', 'x', 'w0', 'w1', 'w2')
MS = 128
GAUSS = 0
PREP_AT = (6, 8, 9)
F32 = jnp.float32


def _dft_consts():
    f = np.arange(C, dtype=np.float64)[:, None] + 0.5
    c = np.arange(C, dtype=np.float64)[None, :]
    th = 2.0 * np.pi * f * c / (2 * C)
    fwd = np.concatenate([np.cos(th), -np.sin(th)], axis=0)
    inv = np.concatenate([np.cos(th).T, -np.sin(th).T], axis=1) / C
    return fwd.astype(np.float32), inv.astype(np.float32)


_FWD, _INV = _dft_consts()
_NT_DIMS = (((1,), (1,)), ((), ()))


def _dot(a, b):
    return jnp.dot(a, b, preferred_element_type=F32)


def _dot_nt(a, b):
    return jax.lax.dot_general(a, b, _NT_DIMS, preferred_element_type=F32)


def _kernel(
    shift_ref, ssmd_ref, gw_ref, mem0_ref, fwd_ref, inv_ref,
    x_hbm, k_hbm, v_hbm, sk_hbm, wq_hbm, wk_hbm, wv_hbm, wo_hbm,
    out_hbm,
    xb, kb, vb, skb,
    yb, kvb,
    kf,
    xsa, ksa, zsa, xsb, ksb, zsb,
    wst,
    wqkv,
    wob,
    ring,
    left,
    ebuf,
    mqkv,
    hyb,
    outb,
    sem_a, sem_w, sem_o,
):
    def a_copies(t):
        return [
            pltpu.make_async_copy(x_hbm.at[:, pl.ds(t * 128, 128)], xb.at[t], sem_a.at[0, t]),
            pltpu.make_async_copy(k_hbm.at[:, pl.ds(t * 128, 128)], kb.at[t], sem_a.at[1, t]),
            pltpu.make_async_copy(v_hbm.at[:, pl.ds(t * 128, 128)], vb.at[t], sem_a.at[2, t]),
            pltpu.make_async_copy(sk_hbm.at[pl.ds(t * 128, 128), :], skb.at[t], sem_a.at[3, t]),
        ]

    whbm = (wq_hbm, wk_hbm, wv_hbm)
    WCH = 4
    DC = D // WCH

    def w_copy(i, c):
        return pltpu.make_async_copy(whbm[i].at[pl.ds(c * DC, DC)], wst.at[i, pl.ds(c * DC, DC)], sem_w.at[i * WCH + c])

    def wo_copy(j):
        return pltpu.make_async_copy(wo_hbm.at[:, pl.ds(j * 128, 128)], wob.at[j], sem_w.at[3 * WCH + j])

    def start_a(t):
        for c in a_copies(t)[1:]:
            c.start()

    def start_w(i):
        for c in range(WCH):
            w_copy(i, c).start()

    def start_x():
        for t in range(NT):
            a_copies(t)[0].start()

    for item in DMA_ORDER:
        if item == 'x':
            start_x()
        elif item[0] == 'w':
            start_w(int(item[1]))
        else:
            start_a(int(item))
    for j in range(NT):
        wo_copy(j).start()

    def relayout_blocks(i, it):
        for b in range(64 // NB):
            d0 = pl.multiple_of(it * (16 * (64 // NB)) + b * 16, 16)
            wqkv[i * H:(i + 1) * H, pl.ds(d0, 16), :] = jnp.swapaxes(wst[i, pl.ds(d0, 16), :, :], 0, 1)

    def first_pass(i):
        if i == 0:
            for t in range(NT):
                a_copies(t)[0].wait()
        xl = jnp.concatenate([xb[t, 0:64, :] for t in range(NT)], axis=1)
        for h in range(H):
            c = i * H + h
            y = _dot(xl, wqkv[c]).astype(BF)
            ring[0, c, :, :] = y[0:32]
            ring[1, c, :, :] = y[32:64]

    fwd = fwd_ref[...]
    inv = inv_ref[...]
    shift = shift_ref[...].astype(F32)
    rowpar = jax.lax.broadcasted_iota(jnp.int32, (8, 128), 0)
    sgn = jnp.where((rowpar & 1) == 0, 1.0, -1.0).astype(F32)

    xbufs = ((xsa, ksa, zsa), (xsb, ksb, zsb))

    def fwd_block(t, j):
        xs, ks, _ = xbufs[t % 2]
        sh = [shift[q:q + 1, t * 128:(t + 1) * 128] for q in range(KS)]
        r0 = pl.multiple_of(j * C, C)
        kcur = kb[t, pl.ds(r0, C), :].astype(F32)
        rp = pl.multiple_of(jnp.maximum(r0 - 16, 0), 16)
        kprev = kb[t, pl.ds(rp, 16), :].astype(F32)
        kf[t % 2, 0:8, :] = jnp.where(j > 0, kprev[8:16], 0.0)
        kf[t % 2, 8:8 + C, :] = kcur
        ksh = kcur * sh[0]
        for q in range(1, KS):
            ksh = ksh + kf[t % 2, 8 - q:8 - q + C, :] * sh[q]
        kvf = ksh * vb[t, pl.ds(r0, C), :].astype(F32)
        kv = kvf.astype(BF)
        xs[j] = jnp.concatenate([_dot(fwd[i * MS:(i + 1) * MS], kv) for i in range(2 * C // MS)], axis=0)
        skt = skb[t, :, pl.ds(r0, C)]
        ks[j] = jnp.concatenate([_dot_nt(fwd[i * MS:(i + 1) * MS], skt) for i in range(2 * C // MS)], axis=0)
        kvb[t, pl.ds(r0, C), :] = kv

    def conv_group(t, g):
        xs, ks, zs = xbufs[t % 2]
        f0 = pl.multiple_of(g * 8, 8)
        xr = [xs[j, pl.ds(f0, 8), :] for j in range(NB)]
        xi = [xs[j, pl.ds(C + f0, 8), :] for j in range(NB)]
        kr = [ks[j, pl.ds(f0, 8), :] for j in range(NB)]
        ki = [ks[j, pl.ds(C + f0, 8), :] for j in range(NB)]
        if GAUSS:
            xs_ = [xr[j] + xi[j] for j in range(NB)]
            kd = [ki[j] - kr[j] for j in range(NB)]
            ke = [ki[j] + kr[j] for j in range(NB)]
        pr = pi = None
        for i in range(NB):
            if GAUSS:
                a1 = xs_[i] * kr[0]
                a2 = xr[i] * kd[0]
                a3 = xi[i] * ke[0]
                for j in range(1, i + 1):
                    a1 = a1 + xs_[i - j] * kr[j]
                    a2 = a2 + xr[i - j] * kd[j]
                    a3 = a3 + xi[i - j] * ke[j]
                yr = a1 - a3
                yi = a1 + a2
            else:
                yr = xr[i] * kr[0] - xi[i] * ki[0]
                yi = xr[i] * ki[0] + xi[i] * kr[0]
                for j in range(1, i + 1):
                    yr = yr + (xr[i - j] * kr[j] - xi[i - j] * ki[j])
                    yi = yi + (xr[i - j] * ki[j] + xi[i - j] * kr[j])
            if i == 0:
                zr, zi = yr, yi
            else:
                zr = yr - sgn * pi
                zi = yi + sgn * pr
            pr, pi = yr, yi
            zs[i, pl.ds(f0, 8), :] = zr
            zs[i, pl.ds(C + f0, 8), :] = zi

    def inv_block(t, i):
        zs = xbufs[t % 2][2]
        r0 = pl.multiple_of(i * C, C)
        zb = zs[i].astype(BF)
        y = jnp.concatenate([_dot(inv[m * MS:(m + 1) * MS], zb) for m in range(C // MS)], axis=0)
        yb[t, pl.ds(r0, C), :] = y.astype(BF)

    for st in range(NT + 2):
        if st < NT:
            cps = a_copies(st)
            cps[1].wait()
            cps[2].wait()
            cps[3].wait()
        if st in PREP_AT:
            for c in range(WCH):
                w_copy(PREP_AT.index(st), c).wait()

        def stage_body(i, carry):
            if st in PREP_AT:
                relayout_blocks(PREP_AT.index(st), i)
            if 0 <= st - 2 < NT:
                inv_block(st - 2, i)
            if 0 <= st - 1 < NT:
                for gg in range(C // 8 // NB):
                    conv_group(st - 1, i * (C // 8 // NB) + gg)
            if st < NT:
                fwd_block(st, i)
            return carry

        jax.lax.fori_loop(0, NB, stage_body, 0, unroll=2)
    for i in range(3):
        first_pass(i)

    for j in range(NT):
        wo_copy(j).wait()

    left[...] = jnp.zeros(left.shape, F32)

    r = jax.lax.broadcasted_iota(jnp.int32, (L, LP), 0)
    cidx = jax.lax.broadcasted_iota(jnp.int32, (L, LP), 1)
    amask = (cidx < L) & ((cidx >= SEG) | (r >= SEG) | (cidx <= r))
    LOG2E = 1.4426950408889634
    scale2 = float(E) ** -0.5 * LOG2E
    neg2 = -1e9 * LOG2E
    fill = jnp.where(cidx < L, neg2, -3.0e38).astype(F32)
    z8 = jnp.zeros((8, 128), F32)

    def attention(q, k, v):
        s = _dot_nt(q, k)[0:L]
        s = jnp.where(amask, s * scale2, fill)
        m = jnp.max(s, axis=-1, keepdims=True)
        p = jnp.exp2(s - m)
        den = jnp.sum(p, axis=-1, keepdims=True)
        pz = jnp.concatenate([p, jnp.zeros((LP - L, LP), F32)], axis=0).astype(BF)
        return _dot(pz, v)[0:L] * (1.0 / den)

    def gate(row0, n):
        acc = None
        for t in range(NT):
            p = xb[t, pl.ds(row0, n), :].astype(F32) * gw_ref[:, t * 128:(t + 1) * 128].astype(F32)
            acc = p if acc is None else acc + p
        return jax.nn.sigmoid(jnp.sum(acc, axis=-1, keepdims=True))

    def combine(j, row0, b, g):
        n = b.shape[0]
        rows = pl.ds(row0, n)
        dd = ssmd_ref[:, j * 128:(j + 1) * 128].astype(F32)
        a = xb[j, rows, :].astype(F32) * (yb[j, rows, :].astype(F32) + kvb[j, rows, :].astype(F32) * dd)
        outb[j, rows, :] = (g * a + (1.0 - g) * b).astype(BF)

    NG = H // G

    def step(even, mem, s, sl, slA, slB, ra, rb):
        nrow = LP if even else 32
        for t in range(NT):
            mt = mem[:, t * 128:(t + 1) * 128]
            extra = xb[t, pl.ds(rb + (24 if even else 16), 8), :].astype(F32)
            hyb[t, :, :] = jnp.concatenate([mt, extra], axis=0).astype(BF)

        def load_lhs():
            parts = []
            for t in range(NT):
                main = xb[t, pl.ds(ra, SEG), :] if even else xb[t, pl.ds(rb, 16), :]
                parts.append(jnp.concatenate([main, hyb[t]], axis=0))
            return jnp.concatenate(parts, axis=1)

        def proj(lhs, h):
            for w in range(3):
                c = w * H + h
                y = _dot(lhs, wqkv[c])
                if even:
                    ring[slA, c, :, :] = y[0:32].astype(BF)
                    ring[slB, c, 24:32, :] = y[40:48].astype(BF)
                    m8 = y[32:40]
                else:
                    ring[slB, c, 0:16, :] = y[0:16].astype(BF)
                    ring[slB, c, 16:24, :] = y[24:32].astype(BF)
                    m8 = y[16:24]
                mqkv[c, :, :] = jnp.concatenate([m8, z8], axis=0).astype(BF)

        def att_load(h):
            return [jnp.concatenate([ring[sl, w * H + h, :, :], mqkv[w * H + h, :, :]], axis=0) for w in range(3)]

        def att(h, qkv):
            o = attention(*qkv)
            if even:
                ebuf[h, :, :] = jnp.concatenate([o, left[h]], axis=0).astype(BF)
            else:
                ebuf[h, 0:32, :] = jnp.concatenate([o[0:16], o[32:40], o[16:24]], axis=0).astype(BF)
                left[h] = o[24:32]

        lhs0 = load_lhs()
        for h in range(G):
            proj(lhs0, h)

        hp = (NG - 1) * G
        ins = [att_load(hp + i) for i in range(G)]
        for i in range(G):
            att(hp + i, ins[i])

        ka = hp * E
        ys = []
        r_cur = pl.multiple_of(s * SEG, SEG)
        if even:
            r_prev = pl.multiple_of(jax.lax.rem(s * SEG + (S - 8), S), 8)
            g_cur = gate(r_cur, 32)
            g_prev = gate(r_prev, 8)
        else:
            r_hi = pl.multiple_of(s * SEG + 16, 8)
            g_cur = gate(r_cur, 16)
            g_hi = gate(r_hi, 8)
        if ka > 0:
            lhsa = jnp.concatenate([ebuf[h, 0:nrow, :] for h in range(hp)], axis=1)
        lhsb = jnp.concatenate([ebuf[h, 0:nrow, :] for h in range(hp, H)], axis=1)
        for j in range(NT):
            y = _dot(lhsb, wob[j, ka:H * E, :])
            if ka > 0:
                y = _dot(lhsa, wob[j, 0:ka, :]) + y
            if even:
                ys.append(y[32:40])
                combine(j, r_cur, y[0:32], g_cur)
                combine(j, r_prev, y[40:48], g_prev)
            else:
                ys.append(y[16:24])
                combine(j, r_cur, y[0:16], g_cur)
                combine(j, r_hi, y[24:32], g_hi)
        return jnp.concatenate(ys, axis=1).astype(BF).astype(F32)

    NOC = 4
    RC = S // NOC

    def out_copy(q, j):
        return pltpu.make_async_copy(outb.at[j, pl.ds(q * RC, RC), :],
                                     out_hbm.at[pl.ds(q * RC, RC), pl.ds(j * 128, 128)], sem_o.at[q, j])

    def pair_body(p, mem):
        for q in range(NOC - 1):
            @pl.when(p == (q + 1) * (NSEG // 2 // NOC) + 1)
            def _():
                for j in range(NT):
                    out_copy(q, j).start()

        s0 = 2 * p
        sl0 = jax.lax.rem(s0, 4)
        sl2 = jax.lax.rem(s0 + 2, 4)
        ra = pl.multiple_of(jnp.minimum(s0 + 2, NSEG - 2) * SEG, SEG)
        rb = pl.multiple_of(ra + SEG, SEG)
        mem = step(True, mem, s0, sl0, sl2, sl2 + 1, ra, rb)
        mem = step(False, mem, s0 + 1, sl0 + 1, sl2, sl2 + 1, ra, rb)
        return mem

    jax.lax.fori_loop(0, NSEG // 2, pair_body, mem0_ref[...].astype(F32))

    g_last = gate(S - 8, 8)
    lhs = jnp.concatenate([jnp.concatenate([left[h], z8], axis=0).astype(BF) for h in range(H)], axis=1)
    for j in range(NT):
        y = _dot(lhs, wob[j])
        combine(j, S - 8, y[0:8], g_last)

    for j in range(NT):
        out_copy(NOC - 1, j).start()
    for q in range(NOC):
        for j in range(NT):
            out_copy(q, j).wait()


@functools.partial(jax.jit, static_argnames=("B_seg_len",))
def pallas_gated_mix__ssm_conv_h3__memory_aug_recurrent_mem_tr__prompt_kernel(
    A_q, A_k, A_v, A_shift_k, A_ssm_k, A_ssm_D, B_x, B_mem0, B_Wq, B_Wk, B_Wv, B_Wo, B_seg_len, gate_w,
):
    del B_x
    assert A_q.shape == (1, S, D) and B_seg_len == SEG and B_mem0.shape == (1, M, D)
    assert B_Wq.shape == (D, H, E) and A_shift_k.shape == (D, KS)
    vm = pl.BlockSpec(memory_space=pltpu.VMEM)
    hbm = pl.BlockSpec(memory_space=pl.ANY)
    out = pl.pallas_call(
        _kernel,
        out_shape=jax.ShapeDtypeStruct((S, D), BF),
        in_specs=[vm] * 6 + [hbm] * 8,
        out_specs=hbm,
        scratch_shapes=[
            pltpu.VMEM((NT, S, 128), BF), pltpu.VMEM((NT, S, 128), BF), pltpu.VMEM((NT, S, 128), BF),
            pltpu.VMEM((NT, 128, S), BF),
            pltpu.VMEM((NT, S, 128), BF), pltpu.VMEM((NT, S, 128), BF),
            pltpu.VMEM((2, 8 + C, 128), F32),
            pltpu.VMEM((NB, 2 * C, 128), F32), pltpu.VMEM((NB, 2 * C, 128), F32), pltpu.VMEM((NB, 2 * C, 128), F32),
            pltpu.VMEM((NB, 2 * C, 128), F32), pltpu.VMEM((NB, 2 * C, 128), F32), pltpu.VMEM((NB, 2 * C, 128), F32),
            pltpu.VMEM((3, D, H, E), BF),
            pltpu.VMEM((3 * H, D, E), BF),
            pltpu.VMEM((NT, H * E, 128), BF),
            pltpu.VMEM((4, 3 * H, SEG, E), BF),
            pltpu.VMEM((H, 8, E), F32),
            pltpu.VMEM((H, LP, E), BF),
            pltpu.VMEM((3 * H, 16, E), BF),
            pltpu.VMEM((NT, 16, 128), BF),
            pltpu.VMEM((NT, S, 128), BF),
            pltpu.SemaphoreType.DMA((4, NT)), pltpu.SemaphoreType.DMA((12 + NT,)), pltpu.SemaphoreType.DMA((4, NT)),
        ],
        compiler_params=pltpu.CompilerParams(vmem_limit_bytes=124 * 1024 * 1024),
    )(
        A_shift_k.T, A_ssm_D.reshape(1, D), gate_w.reshape(1, D), B_mem0.reshape(M, D),
        jnp.asarray(_FWD, BF), jnp.asarray(_INV, BF),
        A_q.reshape(S, D), A_k.reshape(S, D), A_v.reshape(S, D), A_ssm_k,
        B_Wq, B_Wk, B_Wv, B_Wo.reshape(H * E, D),
    )
    return out.reshape(1, S, D)
```

```python
import functools
import numpy as np
import jax
import jax.numpy as jnp
import jax.experimental.pallas as pl
import jax.experimental.pallas.tpu as pltpu

S = 2048
D = 1024
H = 32
E = 128
M = 8
SEG = 32
NSEG = S // SEG
C = 256
NB = S // C
NT = D // 128
KS = 4
L = M + SEG
LP = 48

BF = jnp.bfloat16
G = 32
DMA_ORDER = ('0', '1', '2', '3', '4', '5', '6', '7', 'x', 'w0', 'w1', 'w2')
MS = 128
GAUSS = 0
PREP_AT = (6, 8, 9)
F32 = jnp.float32


def _dft_consts():
    f = np.arange(C, dtype=np.float64)[:, None] + 0.5
    c = np.arange(C, dtype=np.float64)[None, :]
    th = 2.0 * np.pi * f * c / (2 * C)
    fwd = np.concatenate([np.cos(th), -np.sin(th)], axis=0)
    inv = np.concatenate([np.cos(th).T, -np.sin(th).T], axis=1) / C
    return fwd.astype(np.float32), inv.astype(np.float32)


_FWD, _INV = _dft_consts()
_NT_DIMS = (((1,), (1,)), ((), ()))


def _dot(a, b):
    return jnp.dot(a, b, preferred_element_type=F32)


def _dot_nt(a, b):
    return jax.lax.dot_general(a, b, _NT_DIMS, preferred_element_type=F32)


def _kernel(
    shift_ref, ssmd_ref, gw_ref, mem0_ref, fwd_ref, inv_ref,
    x_hbm, k_hbm, v_hbm, sk_hbm, wq_hbm, wk_hbm, wv_hbm, wo_hbm,
    out_hbm,
    xb, kb, vb, skb,
    yb, kvb,
    kf,
    xsa, ksa, zsa, xsb, ksb, zsb,
    wst,
    wqkv,
    wob,
    ring,
    left,
    ebuf,
    mqkv,
    hyb,
    outb,
    sem_a, sem_w, sem_o,
):
    def a_copy(kind, t):
        cols = pl.ds(t * 128, 128)
        if kind == 3:
            return pltpu.make_async_copy(sk_hbm.at[cols, :], skb.at[t], sem_a.at[3, t])
        src_ref, dst_ref = ((x_hbm, xb), (k_hbm, kb), (v_hbm, vb))[kind]
        return pltpu.make_async_copy(src_ref.at[:, cols], dst_ref.at[t], sem_a.at[kind, t])

    whbm = (wq_hbm, wk_hbm, wv_hbm)
    WCH = 4
    DC = D // WCH

    def w_copy(i, c):
        return pltpu.make_async_copy(whbm[i].at[pl.ds(c * DC, DC)], wst.at[i, pl.ds(c * DC, DC)], sem_w.at[i * WCH + c])

    def wo_copy(j):
        return pltpu.make_async_copy(wo_hbm.at[:, pl.ds(j * 128, 128)], wob.at[j], sem_w.at[3 * WCH + j])

    def start_a(t):
        for kind in (1, 2, 3):
            a_copy(kind, t).start()

    def start_w(i):
        for c in range(WCH):
            w_copy(i, c).start()

    def start_x():
        for t in range(NT):
            a_copy(0, t).start()

    for item in DMA_ORDER:
        if item == 'x':
            start_x()
        elif item[0] == 'w':
            start_w(int(item[1]))
        else:
            start_a(int(item))
    for j in range(NT):
        wo_copy(j).start()

    def relayout_blocks(i, it):
        for b in range(64 // NB):
            d0 = pl.multiple_of(it * (16 * (64 // NB)) + b * 16, 16)
            wqkv[i * H:(i + 1) * H, pl.ds(d0, 16), :] = jnp.swapaxes(wst[i, pl.ds(d0, 16), :, :], 0, 1)

    def first_pass(i):
        if i == 0:
            for t in range(NT):
                a_copy(0, t).wait()
        xl = jnp.concatenate([xb[t, 0:64, :] for t in range(NT)], axis=1)
        for h in range(H):
            c = i * H + h
            y = _dot(xl, wqkv[c]).astype(BF)
            ring[0, c, :, :] = y[0:32]
            ring[1, c, :, :] = y[32:64]

    fwd = fwd_ref[...]
    inv = inv_ref[...]
    shift = shift_ref[...].astype(F32)
    rowpar = jax.lax.broadcasted_iota(jnp.int32, (8, 128), 0)
    sgn = jnp.where((rowpar & 1) == 0, 1.0, -1.0).astype(F32)

    xbufs = ((xsa, ksa, zsa), (xsb, ksb, zsb))

    def fwd_block(t, j):
        xs, ks, _ = xbufs[t % 2]
        sh = [shift[q:q + 1, t * 128:(t + 1) * 128] for q in range(KS)]
        r0 = pl.multiple_of(j * C, C)
        kcur = kb[t, pl.ds(r0, C), :].astype(F32)
        rp = pl.multiple_of(jnp.maximum(r0 - 16, 0), 16)
        kprev = kb[t, pl.ds(rp, 16), :].astype(F32)
        kf[t % 2, 0:8, :] = jnp.where(j > 0, kprev[8:16], 0.0)
        kf[t % 2, 8:8 + C, :] = kcur
        ksh = kcur * sh[0]
        for q in range(1, KS):
            ksh = ksh + kf[t % 2, 8 - q:8 - q + C, :] * sh[q]
        kvf = ksh * vb[t, pl.ds(r0, C), :].astype(F32)
        kv = kvf.astype(BF)
        xs[j] = jnp.concatenate([_dot(fwd[i * MS:(i + 1) * MS], kv) for i in range(2 * C // MS)], axis=0)
        skt = skb[t, :, pl.ds(r0, C)]
        ks[j] = jnp.concatenate([_dot_nt(fwd[i * MS:(i + 1) * MS], skt) for i in range(2 * C // MS)], axis=0)
        kvb[t, pl.ds(r0, C), :] = kv

    def conv_group(t, g):
        xs, ks, zs = xbufs[t % 2]
        f0 = pl.multiple_of(g * 8, 8)
        xr = [xs[j, pl.ds(f0, 8), :] for j in range(NB)]
        xi = [xs[j, pl.ds(C + f0, 8), :] for j in range(NB)]
        kr = [ks[j, pl.ds(f0, 8), :] for j in range(NB)]
        ki = [ks[j, pl.ds(C + f0, 8), :] for j in range(NB)]
        if GAUSS:
            xs_ = [xr[j] + xi[j] for j in range(NB)]
            kd = [ki[j] - kr[j] for j in range(NB)]
            ke = [ki[j] + kr[j] for j in range(NB)]
        pr = pi = None
        for i in range(NB):
            if GAUSS:
                a1 = xs_[i] * kr[0]
                a2 = xr[i] * kd[0]
                a3 = xi[i] * ke[0]
                for j in range(1, i + 1):
                    a1 = a1 + xs_[i - j] * kr[j]
                    a2 = a2 + xr[i - j] * kd[j]
                    a3 = a3 + xi[i - j] * ke[j]
                yr = a1 - a3
                yi = a1 + a2
            else:
                yr = xr[i] * kr[0] - xi[i] * ki[0]
                yi = xr[i] * ki[0] + xi[i] * kr[0]
                for j in range(1, i + 1):
                    yr = yr + (xr[i - j] * kr[j] - xi[i - j] * ki[j])
                    yi = yi + (xr[i - j] * ki[j] + xi[i - j] * kr[j])
            if i == 0:
                zr, zi = yr, yi
            else:
                zr = yr - sgn * pi
                zi = yi + sgn * pr
            pr, pi = yr, yi
            zs[i, pl.ds(f0, 8), :] = zr
            zs[i, pl.ds(C + f0, 8), :] = zi

    def inv_block(t, i):
        zs = xbufs[t % 2][2]
        r0 = pl.multiple_of(i * C, C)
        zb = zs[i].astype(BF)
        y = jnp.concatenate([_dot(inv[m * MS:(m + 1) * MS], zb) for m in range(C // MS)], axis=0)
        yb[t, pl.ds(r0, C), :] = y.astype(BF)

    for st in range(NT + 2):
        if st < NT:
            for kind in (1, 2, 3):
                a_copy(kind, st).wait()
        if st in PREP_AT:
            for c in range(WCH):
                w_copy(PREP_AT.index(st), c).wait()

        def stage_body(i, carry):
            if st in PREP_AT:
                relayout_blocks(PREP_AT.index(st), i)
            if 0 <= st - 2 < NT:
                inv_block(st - 2, i)
            if 0 <= st - 1 < NT:
                for gg in range(C // 8 // NB):
                    conv_group(st - 1, i * (C // 8 // NB) + gg)
            if st < NT:
                fwd_block(st, i)
            return carry

        jax.lax.fori_loop(0, NB, stage_body, 0, unroll=2)
    for i in range(3):
        first_pass(i)

    for j in range(NT):
        wo_copy(j).wait()

    left[...] = jnp.zeros(left.shape, F32)

    r = jax.lax.broadcasted_iota(jnp.int32, (L, LP), 0)
    cidx = jax.lax.broadcasted_iota(jnp.int32, (L, LP), 1)
    amask = (cidx < L) & ((cidx >= SEG) | (r >= SEG) | (cidx <= r))
    LOG2E = 1.4426950408889634
    scale2 = float(E) ** -0.5 * LOG2E
    neg2 = -1e9 * LOG2E
    fill = jnp.where(cidx < L, neg2, -3.0e38).astype(F32)
    z8 = jnp.zeros((8, 128), F32)

    def attention(q, k, v):
        s = _dot_nt(q, k)[0:L]
        s = jnp.where(amask, s * scale2, fill)
        m = jnp.max(s, axis=-1, keepdims=True)
        p = jnp.exp2(s - m)
        den = jnp.sum(p, axis=-1, keepdims=True)
        pz = jnp.concatenate([p, jnp.zeros((LP - L, LP), F32)], axis=0).astype(BF)
        return _dot(pz, v)[0:L] * (1.0 / den)

    def gate(row0, n):
        acc = None
        for t in range(NT):
            p = xb[t, pl.ds(row0, n), :].astype(F32) * gw_ref[:, t * 128:(t + 1) * 128].astype(F32)
            acc = p if acc is None else acc + p
        return jax.nn.sigmoid(jnp.sum(acc, axis=-1, keepdims=True))

    def combine(j, row0, b, g):
        n = b.shape[0]
        rows = pl.ds(row0, n)
        dd = ssmd_ref[:, j * 128:(j + 1) * 128].astype(F32)
        a = xb[j, rows, :].astype(F32) * (yb[j, rows, :].astype(F32) + kvb[j, rows, :].astype(F32) * dd)
        outb[j, rows, :] = (g * a + (1.0 - g) * b).astype(BF)

    NG = H // G

    def step(even, mem, s, sl, slA, slB, ra, rb):
        nrow = LP if even else 32
        for t in range(NT):
            mt = mem[:, t * 128:(t + 1) * 128]
            extra = xb[t, pl.ds(rb + (24 if even else 16), 8), :].astype(F32)
            hyb[t, :, :] = jnp.concatenate([mt, extra], axis=0).astype(BF)

        def load_lhs():
            parts = []
            for t in range(NT):
                main = xb[t, pl.ds(ra, SEG), :] if even else xb[t, pl.ds(rb, 16), :]
                parts.append(jnp.concatenate([main, hyb[t]], axis=0))
            return jnp.concatenate(parts, axis=1)

        def proj(lhs, h):
            for w in range(3):
                c = w * H + h
                y = _dot(lhs, wqkv[c])
                if even:
                    ring[slA, c, :, :] = y[0:32].astype(BF)
                    ring[slB, c, 24:32, :] = y[40:48].astype(BF)
                    m8 = y[32:40]
                else:
                    ring[slB, c, 0:16, :] = y[0:16].astype(BF)
                    ring[slB, c, 16:24, :] = y[24:32].astype(BF)
                    m8 = y[16:24]
                mqkv[c, :, :] = jnp.concatenate([m8, z8], axis=0).astype(BF)

        def att_load(h):
            return [jnp.concatenate([ring[sl, w * H + h, :, :], mqkv[w * H + h, :, :]], axis=0) for w in range(3)]

        def att(h, qkv):
            o = attention(*qkv)
            if even:
                ebuf[h, :, :] = jnp.concatenate([o, left[h]], axis=0).astype(BF)
            else:
                ebuf[h, 0:32, :] = jnp.concatenate([o[0:16], o[32:40], o[16:24]], axis=0).astype(BF)
                left[h] = o[24:32]

        lhs0 = load_lhs()
        for h in range(G):
            proj(lhs0, h)

        hp = (NG - 1) * G
        ins = [att_load(hp + i) for i in range(G)]
        for i in range(G):
            att(hp + i, ins[i])

        ka = hp * E
        ys = []
        r_cur = pl.multiple_of(s * SEG, SEG)
        if even:
            r_prev = pl.multiple_of(jax.lax.rem(s * SEG + (S - 8), S), 8)
            g_cur = gate(r_cur, 32)
            g_prev = gate(r_prev, 8)
        else:
            r_hi = pl.multiple_of(s * SEG + 16, 8)
            g_cur = gate(r_cur, 16)
            g_hi = gate(r_hi, 8)
        if ka > 0:
            lhsa = jnp.concatenate([ebuf[h, 0:nrow, :] for h in range(hp)], axis=1)
        lhsb = jnp.concatenate([ebuf[h, 0:nrow, :] for h in range(hp, H)], axis=1)
        for j in range(NT):
            y = _dot(lhsb, wob[j, ka:H * E, :])
            if ka > 0:
                y = _dot(lhsa, wob[j, 0:ka, :]) + y
            if even:
                ys.append(y[32:40])
                combine(j, r_cur, y[0:32], g_cur)
                combine(j, r_prev, y[40:48], g_prev)
            else:
                ys.append(y[16:24])
                combine(j, r_cur, y[0:16], g_cur)
                combine(j, r_hi, y[24:32], g_hi)
        return jnp.concatenate(ys, axis=1).astype(BF).astype(F32)

    NOC = 4
    RC = S // NOC

    def out_copy(q, j):
        return pltpu.make_async_copy(outb.at[j, pl.ds(q * RC, RC), :],
                                     out_hbm.at[pl.ds(q * RC, RC), pl.ds(j * 128, 128)], sem_o.at[q, j])

    def pair_body(p, mem):
        for q in range(NOC - 1):
            @pl.when(p == (q + 1) * (NSEG // 2 // NOC) + 1)
            def _():
                for j in range(NT):
                    out_copy(q, j).start()

        s0 = 2 * p
        sl0 = jax.lax.rem(s0, 4)
        sl2 = jax.lax.rem(s0 + 2, 4)
        ra = pl.multiple_of(jnp.minimum(s0 + 2, NSEG - 2) * SEG, SEG)
        rb = pl.multiple_of(ra + SEG, SEG)
        mem = step(True, mem, s0, sl0, sl2, sl2 + 1, ra, rb)
        mem = step(False, mem, s0 + 1, sl0 + 1, sl2, sl2 + 1, ra, rb)
        return mem

    jax.lax.fori_loop(0, NSEG // 2, pair_body, mem0_ref[...].astype(F32))

    g_last = gate(S - 8, 8)
    lhs = jnp.concatenate([jnp.concatenate([left[h], z8], axis=0).astype(BF) for h in range(H)], axis=1)
    for j in range(NT):
        y = _dot(lhs, wob[j])
        combine(j, S - 8, y[0:8], g_last)

    for j in range(NT):
        out_copy(NOC - 1, j).start()
    for q in range(NOC):
        for j in range(NT):
            out_copy(q, j).wait()


@functools.partial(jax.jit, static_argnames=("B_seg_len",))
def pallas_gated_mix__ssm_conv_h3__memory_aug_recurrent_mem_tr__prompt_kernel(
    A_q, A_k, A_v, A_shift_k, A_ssm_k, A_ssm_D, B_x, B_mem0, B_Wq, B_Wk, B_Wv, B_Wo, B_seg_len, gate_w,
):
    del B_x
    assert A_q.shape == (1, S, D) and B_seg_len == SEG and B_mem0.shape == (1, M, D)
    assert B_Wq.shape == (D, H, E) and A_shift_k.shape == (D, KS)
    vm = pl.BlockSpec(memory_space=pltpu.VMEM)
    hbm = pl.BlockSpec(memory_space=pl.ANY)
    out = pl.pallas_call(
        _kernel,
        out_shape=jax.ShapeDtypeStruct((S, D), BF),
        in_specs=[vm] * 6 + [hbm] * 8,
        out_specs=hbm,
        scratch_shapes=[
            pltpu.VMEM((NT, S, 128), BF), pltpu.VMEM((NT, S, 128), BF), pltpu.VMEM((NT, S, 128), BF),
            pltpu.VMEM((NT, 128, S), BF),
            pltpu.VMEM((NT, S, 128), BF), pltpu.VMEM((NT, S, 128), BF),
            pltpu.VMEM((2, 8 + C, 128), F32),
            pltpu.VMEM((NB, 2 * C, 128), F32), pltpu.VMEM((NB, 2 * C, 128), F32), pltpu.VMEM((NB, 2 * C, 128), F32),
            pltpu.VMEM((NB, 2 * C, 128), F32), pltpu.VMEM((NB, 2 * C, 128), F32), pltpu.VMEM((NB, 2 * C, 128), F32),
            pltpu.VMEM((3, D, H, E), BF),
            pltpu.VMEM((3 * H, D, E), BF),
            pltpu.VMEM((NT, H * E, 128), BF),
            pltpu.VMEM((4, 3 * H, SEG, E), BF),
            pltpu.VMEM((H, 8, E), F32),
            pltpu.VMEM((H, LP, E), BF),
            pltpu.VMEM((3 * H, 16, E), BF),
            pltpu.VMEM((NT, 16, 128), BF),
            pltpu.VMEM((NT, S, 128), BF),
            pltpu.SemaphoreType.DMA((4, NT)), pltpu.SemaphoreType.DMA((12 + NT,)), pltpu.SemaphoreType.DMA((4, NT)),
        ],
        compiler_params=pltpu.CompilerParams(vmem_limit_bytes=124 * 1024 * 1024),
    )(
        A_shift_k.T, A_ssm_D.reshape(1, D), gate_w.reshape(1, D), B_mem0.reshape(M, D),
        jnp.asarray(_FWD, BF), jnp.asarray(_INV, BF),
        A_q.reshape(S, D), A_k.reshape(S, D), A_v.reshape(S, D), A_ssm_k,
        B_Wq, B_Wk, B_Wv, B_Wo.reshape(H * E, D),
    )
    return out.reshape(1, S, D)
```
